```python
import os as _os
_os.environ.setdefault('JAX_PLATFORMS', 'cpu')
import jax
import jax.numpy as jnp

def _softmax(x, axis=-1):
    return jax.nn.softmax(x, axis=axis)

def _gelu(x):
    return jax.nn.gelu(x, approximate=True)

def _silu(x):
    return jax.nn.silu(x)

def _sigmoid(x):
    return jax.nn.sigmoid(x)

def _layernorm(x, axis=-1, eps=1e-05):
    m = jnp.mean(x, axis=axis, keepdims=True)
    v = jnp.var(x, axis=axis, keepdims=True)
    return (x - m) / jnp.sqrt(v + eps)

def _scatter_add(tgt, idx, src, axis=0):
    return tgt.at[idx].add(src)

def _segment_sum(src, seg, n):
    return jax.ops.segment_sum(src, seg, n)

class _Rng:

    def __init__(self, key):
        self._k = key

    def _next(self):
        self._k, sub = jax.random.split(self._k)
        return sub

    def normal(self, shape):
        return jax.random.normal(self._next(), shape, dtype=jnp.bfloat16)

    def randint(self, lo, hi, shape):
        return jax.random.randint(self._next(), shape, lo, hi, dtype=jnp.int32)

    def uniform(self, shape, lo=0.0, hi=1.0):
        return jax.random.uniform(self._next(), shape, jnp.bfloat16, lo, hi)

    def permutation(self, n):
        return jax.random.permutation(self._next(), n)
kernel_name = 'adaLN_cond__mha_block__dense_activation_squared_relu__prompt'

def setup_inputs():
    _rng = _Rng(jax.random.key(int.from_bytes(__import__("os").urandom(4), "little")))
    _w = lambda a: (lambda t: t.astype(jnp.bfloat16) if jnp.issubdtype(t.dtype, jnp.floating) else t)(jnp.asarray(a))

    def _A_setup():
        B, S, D, H = (1, 2048, 512, 32)
        return {'x': _w((lambda *s: _rng.normal(s) * 0.05)(B, S, D)), 'wqkv': _w((lambda *s: _rng.normal(s) * 0.1)(D, 3 * D)), 'wo': _w((lambda *s: _rng.normal(s) * 0.05)(D, D))}
    _A_in = _A_setup()

    def _B_setup():
        B, S, D, F = (1, 2048, 512, 1792)
        return {'x': _w((lambda *s: _rng.normal(s) * 0.05)(B, S, D)), 'w1': _w((lambda *s: _rng.normal(s) * 0.05)(D, F)), 'b1': _w((lambda *s: _rng.normal(s) * 0.05)(F)), 'w2': _w((lambda *s: _rng.normal(s) * 0.05)(F, D)), 'b2': _w((lambda *s: _rng.normal(s) * 0.05)(D))}
    _B_in = _B_setup()
    return {'A_x': _A_in['x'], 'A_wqkv': _A_in['wqkv'], 'A_wo': _A_in['wo'], 'B_x': _B_in['x'], 'B_w1': _B_in['w1'], 'B_b1': _B_in['b1'], 'B_w2': _B_in['w2'], 'B_b2': _B_in['b2'], 'c': _w((lambda *s: _rng.normal(s) * 0.05)(1, 512) * 8.0), 'w_mod': _w((lambda *s: _rng.normal(s) * 0.05)(512, 6 * 512) * 512 ** (-0.5) * 8.0)}

def reference(A_x, A_wqkv, A_wo, B_x, B_w1, B_b1, B_w2, B_b2, c, w_mod):

    def _A_ref(x, wqkv, wo):
        B, S, D = x.shape
        H = 32
        Dh = D // H
        qkv = (lambda x, *d: x.transpose(*d))((x @ wqkv).reshape(B, S, 3, H, Dh), 2, 0, 3, 1, 4)
        q, k, v = (qkv[0], qkv[1], qkv[2])
        scores = jnp.einsum('bhqd,bhkd->bhqk', q, k) * Dh ** (-0.5)
        p = _softmax(scores, axis=-1)
        o = jnp.einsum('bhqk,bhkd->bhqd', p, v)
        return (lambda x, *d: x.transpose(*d))(o, 0, 2, 1, 3).reshape(B, S, D) @ wo

    def _B_ref(x, w1, b1, w2, b2):
        h = jnp.einsum('bsd,df->bsf', x, w1) + b1
        zero = jnp.zeros_like(h)
        r = jnp.where(h > zero, h, zero)
        h = r * r
        out = jnp.einsum('bsf,fd->bsd', h, w2) + b2
        return out
    x = A_x
    mod = (_silu(c) @ w_mod).reshape(c.shape[0], 6, 1, -1)
    sa, ca, ga, sb, cb, gb = (mod[:, 0].copy(), mod[:, 1].copy(), mod[:, 2].copy(), mod[:, 3].copy(), mod[:, 4].copy(), mod[:, 5].copy())
    h = _layernorm(x, axis=-1) * (1 + ca) + sa
    x = x + ga * _A_ref(h, A_wqkv, A_wo)
    h = _layernorm(x, axis=-1) * (1 + cb) + sb
    x = x + gb * _B_ref(h, B_w1, B_b1, B_w2, B_b2)
    return x
```

```python
import jax
import jax.numpy as jnp
import jax.experimental.pallas as pl
import jax.experimental.pallas.tpu as pltpu

BF16 = jnp.bfloat16
F32 = jnp.float32
LOG2E = 1.4426950408889634

N_HEADS = 32
XC = 512
BQ = 1024
BK = 128
HPI = 2
SAFE_RANGE = 200.0
SAFE_VMAX = 32768.0


def _ln(x):
    mu = jnp.mean(x, axis=-1, keepdims=True)
    xc = x - mu
    var = jnp.mean(xc * xc, axis=-1, keepdims=True)
    return xc * jax.lax.rsqrt(var + 1e-5)


def _nt(a, b):
    return jax.lax.dot_general(a, b, (((1,), (1,)), ((), ())), preferred_element_type=F32)


def _kernel(x_hbm, wqkv_hbm, wo_hbm, w1_hbm, b1_ref, w2_hbm, b2_ref, c_ref, wmod_hbm,
            out_hbm,
            x_s, wqkv_s, wo_s, w1_s, w2_s, wmod_s, h_s, k_s, qT_s, vT_s, oT_s,
            qp0, qp1, m_s, out_s, sems, osems, *, S, D, F, force_slow=False):
    nx = S // XC
    dh = D // N_HEADS
    hpg = 128 // dh

    cp_mod0 = pltpu.make_async_copy(wmod_hbm.at[:, pl.ds(0, 2 * D)], wmod_s.at[:, pl.ds(0, 2 * D)], sems.at[0])
    cp_qkv = pltpu.make_async_copy(wqkv_hbm, wqkv_s, sems.at[1])
    cp_x = [pltpu.make_async_copy(x_hbm.at[pl.ds(i * XC, XC)], x_s.at[pl.ds(i * XC, XC)], sems.at[2 + i])
            for i in range(nx)]
    cp_mod1 = pltpu.make_async_copy(wmod_hbm.at[:, pl.ds(2 * D, 4 * D)], wmod_s.at[:, pl.ds(2 * D, 4 * D)],
                                    sems.at[2 + nx])
    cp_wo = pltpu.make_async_copy(wo_hbm, wo_s, sems.at[3 + nx])
    cp_w1 = pltpu.make_async_copy(w1_hbm, w1_s, sems.at[4 + nx])
    cp_w2 = pltpu.make_async_copy(w2_hbm, w2_s, sems.at[5 + nx])
    cp_x[0].start()
    cp_mod0.start()
    cp_qkv.start()
    for i in range(1, nx):
        cp_x[i].start()

    cf = c_ref[...].astype(F32)
    sc = cf * jax.nn.sigmoid(cf)
    sc8 = jnp.broadcast_to(sc, (8, D)).astype(BF16)
    cp_mod0.wait()
    mod0 = jnp.dot(sc8, wmod_s[:, 0:2 * D], preferred_element_type=F32)[0:1]
    sa = mod0[:, 0:D]
    ca1 = 1.0 + mod0[:, D:2 * D]

    cp_qkv.wait()
    wqT = wqkv_s[:, 0:D].T
    wvT = wqkv_s[:, 2 * D:3 * D].T
    wqvT = jnp.concatenate([wqT, wvT], axis=0)
    qscale = (dh ** -0.5) * LOG2E

    r_id = jax.lax.broadcasted_iota(jnp.int32, (N_HEADS, D), 0)
    c_id = jax.lax.broadcasted_iota(jnp.int32, (N_HEADS, D), 1)
    emask = (c_id // dh) == r_id
    e_mat = jnp.where(emask, 1.0, 0.0).astype(BF16)

    ksum = jnp.zeros((8, D), F32)
    kn_max = jnp.zeros((N_HEADS, 128), F32)
    vmax = jnp.zeros((8, 128), F32)
    for i in range(nx):
        cp_x[i].wait()
        rows = pl.ds(i * XC, XC)
        hb = (_ln(x_s[rows, :].astype(F32)) * ca1 + sa).astype(BF16)
        kf = jnp.dot(hb, wqkv_s[:, D:2 * D], preferred_element_type=F32)
        qv = _nt(wqvT, hb)
        kb = kf.astype(BF16)
        k_s[rows, :] = kb
        qf = qv[0:D] * qscale
        qb = qf.astype(BF16)
        qT_s[:, rows] = qb
        vb = qv[D:2 * D].astype(BF16)
        vT_s[:, rows] = vb
        kb32 = kb.astype(F32)
        ksum = ksum + kb32.reshape(XC // 8, 8, D).sum(axis=0)
        kn2 = _nt(e_mat, (kb32 * kb32).astype(BF16))
        for t in range(XC // 128):
            kn_max = jnp.maximum(kn_max, kn2[:, t * 128:(t + 1) * 128])
        qb32 = qb.astype(F32)
        qn2 = jnp.dot(e_mat, (qb32 * qb32).astype(BF16), preferred_element_type=F32)
        m_s[:, rows] = qn2
        va = jnp.abs(vb.astype(F32))
        for t in range(XC // 128):
            vmax = jnp.maximum(vmax, va[:, t * 128:(t + 1) * 128].reshape(D // 8, 8, 128).max(axis=0))
        if i == 0:
            cp_mod1.start()
            cp_wo.start()
            cp_w1.start()
            cp_w2.start()

    kbar = jnp.sum(ksum, axis=0, keepdims=True) * (1.0 / S)
    ek = jnp.where(emask, jnp.broadcast_to(kbar, (N_HEADS, D)), 0.0).astype(BF16)
    kn = jnp.max(kn_max, axis=1, keepdims=True)
    ub = jnp.sqrt(m_s[...] * kn) * 1.02 + 1e-3
    lb = jnp.dot(ek, qT_s[...], preferred_element_type=F32) - ub * (1.0 / 64.0)
    m_s[...] = 0.5 * (ub + lb)
    spread = jnp.max(jnp.max(ub - lb, axis=1, keepdims=True), axis=0, keepdims=True)
    vm = jnp.max(jnp.max(vmax, axis=1, keepdims=True), axis=0, keepdims=True)
    ok = jnp.logical_and(spread <= SAFE_RANGE, vm <= SAFE_VMAX)
    safe = jnp.where(ok, 1, 0)[0, 0] > (1 if force_slow else 0)

    def prep(buf, h):
        hh = h % hpg
        buf[pl.ds(pl.multiple_of(((hh + hpg - 2) % hpg) * dh, dh), dh), :] = jnp.zeros((dh, S), BF16)
        buf[pl.ds(pl.multiple_of(hh * dh, dh), dh), :] = qT_s[pl.ds(pl.multiple_of(h * dh, dh), dh), :]

    qp0[...] = jnp.zeros((128, S), BF16)
    qp1[...] = jnp.zeros((128, S), BF16)

    @pl.when(safe)
    def _fast():
        nq = S // BQ
        nk = S // BK
        bufs = (qp0, qp1)
        prep(qp0, 0)

        def head(h, buf):
            g0 = pl.multiple_of((h // hpg) * 128, 128)
            h0 = pl.multiple_of(h * dh, dh)
            items = [(j, c) for j in range(nq) for c in range(nk)]

            def qk(it):
                j, c = it
                return jnp.dot(k_s[pl.ds(c * BK, BK), pl.ds(g0, 128)], buf[:, j * BQ:(j + 1) * BQ],
                               preferred_element_type=F32)

            acc = None
            l = None
            pend = qk(items[0])
            for i, (j, c) in enumerate(items):
                sT = pend
                if i + 1 < len(items):
                    pend = qk(items[i + 1])
                p = jnp.exp2(sT - m_s[pl.ds(h, 1), j * BQ:(j + 1) * BQ])
                ps = p.reshape(BK // 8, 8, BQ).sum(axis=0)
                pv = jnp.dot(vT_s[pl.ds(h0, dh), pl.ds(c * BK, BK)], p.astype(BF16), preferred_element_type=F32)
                l = ps if c == 0 else l + ps
                acc = pv if c == 0 else acc + pv
                if c == nk - 1:
                    lt = jnp.sum(l, axis=0, keepdims=True)
                    oT_s[pl.ds(h0, dh), j * BQ:(j + 1) * BQ] = (acc / lt).astype(BF16)

        def body(it, carry):
            for u in range(HPI):
                h = it * HPI + u
                prep(bufs[(u + 1) % 2], jnp.minimum(h + 1, N_HEADS - 1))
                head(h, bufs[u % 2])
            return carry

        jax.lax.fori_loop(0, N_HEADS // HPI, body, 0)

    @pl.when(jnp.logical_not(safe))
    def _slow():
        bq, bk = 512, 256

        def hq_body(it, carry):
            h = it // (S // bq)
            j = it % (S // bq)
            g0 = pl.multiple_of((h // hpg) * 128, 128)
            h0 = pl.multiple_of(h * dh, dh)
            q0 = pl.multiple_of(j * bq, bq)
            qp0[:, 0:bq] = jnp.zeros((128, bq), BF16)
            qp0[pl.ds(pl.multiple_of((h % hpg) * dh, dh), dh), 0:bq] = qT_s[pl.ds(h0, dh), pl.ds(q0, bq)]

            def k_body(c, st):
                m, l, acc = st
                k0 = pl.multiple_of(c * bk, bk)
                sT = jnp.dot(k_s[pl.ds(k0, bk), pl.ds(g0, 128)], qp0[:, 0:bq], preferred_element_type=F32)
                m_new = jnp.maximum(m, jnp.max(sT, axis=0, keepdims=True))
                alpha = jnp.exp2(m - m_new)
                p = jnp.exp2(sT - m_new)
                l = l * alpha + jnp.sum(p, axis=0, keepdims=True)
                acc = acc * alpha + jnp.dot(vT_s[pl.ds(h0, dh), pl.ds(k0, bk)], p.astype(BF16),
                                            preferred_element_type=F32)
                return m_new, l, acc

            m0 = jnp.full((1, bq), -jnp.inf, F32)
            _, l, acc = jax.lax.fori_loop(0, S // bk, k_body,
                                          (m0, jnp.zeros((1, bq), F32), jnp.zeros((dh, bq), F32)))
            oT_s[pl.ds(h0, dh), pl.ds(q0, bq)] = (acc / l).astype(BF16)
            return carry

        jax.lax.fori_loop(0, N_HEADS * (S // bq), hq_body, 0)

    cp_mod1.wait()
    mod1 = jnp.dot(sc8, wmod_s[:, 2 * D:6 * D], preferred_element_type=F32)[0:1]
    ga = mod1[:, 0:D]
    sb = mod1[:, D:2 * D]
    cb1 = 1.0 + mod1[:, 2 * D:3 * D]
    gb = mod1[:, 3 * D:4 * D]
    b1 = b1_ref[...].astype(F32)
    b2 = b2_ref[...].astype(F32)
    cp_wo.wait()
    cp_w1.wait()
    cp_w2.wait()

    ocp = []
    for i in range(nx):
        rows = pl.ds(i * XC, XC)
        o = oT_s[:, rows].T
        a = jnp.dot(o, wo_s[...], preferred_element_type=F32)
        x1 = x_s[rows, :].astype(F32) + ga * a
        h2 = (_ln(x1) * cb1 + sb).astype(BF16)
        u = jnp.maximum(jnp.dot(h2, w1_s[...], preferred_element_type=F32) + b1, 0.0)
        u = (u * u).astype(BF16)
        y = jnp.dot(u, w2_s[...], preferred_element_type=F32) + b2
        out_s[rows, :] = (x1 + gb * y).astype(BF16)
        cp = pltpu.make_async_copy(out_s.at[rows], out_hbm.at[rows], osems.at[i])
        cp.start()
        ocp.append(cp)
    for cp in ocp:
        cp.wait()


def _build(S, D, F, force_slow=False):
    import functools
    nx = S // XC
    any_spec = pl.BlockSpec(memory_space=pl.ANY)
    vmem_spec = pl.BlockSpec(memory_space=pltpu.VMEM)
    return pl.pallas_call(
        functools.partial(_kernel, S=S, D=D, F=F, force_slow=force_slow),
        out_shape=jax.ShapeDtypeStruct((S, D), BF16),
        in_specs=[any_spec, any_spec, any_spec, any_spec, vmem_spec, any_spec, vmem_spec, vmem_spec, any_spec],
        out_specs=any_spec,
        scratch_shapes=[
            pltpu.VMEM((S, D), BF16),
            pltpu.VMEM((D, 3 * D), BF16),
            pltpu.VMEM((D, D), BF16),
            pltpu.VMEM((D, F), BF16),
            pltpu.VMEM((F, D), BF16),
            pltpu.VMEM((D, 6 * D), BF16),
            pltpu.VMEM((8, 128), BF16),
            pltpu.VMEM((S, D), BF16),
            pltpu.VMEM((D, S), BF16),
            pltpu.VMEM((D, S), BF16),
            pltpu.VMEM((D, S), BF16),
            pltpu.VMEM((128, S), BF16),
            pltpu.VMEM((128, S), BF16),
            pltpu.VMEM((N_HEADS, S), F32),
            pltpu.VMEM((S, D), BF16),
            pltpu.SemaphoreType.DMA((6 + nx,)),
            pltpu.SemaphoreType.DMA((nx,)),
        ],
        compiler_params=pltpu.CompilerParams(vmem_limit_bytes=100 * 2 ** 20),
        name="adaln_block",
    )


@jax.jit
def pallas_adaLN_cond__mha_block__dense_activation_squared_relu__prompt_kernel(
    A_x: jax.Array,
    A_wqkv: jax.Array,
    A_wo: jax.Array,
    B_x: jax.Array,
    B_w1: jax.Array,
    B_b1: jax.Array,
    B_w2: jax.Array,
    B_b2: jax.Array,
    c: jax.Array,
    w_mod: jax.Array,
):
    del B_x
    B, S, D = A_x.shape
    F = B_w1.shape[1]
    out = _build(S, D, F)(
        A_x.reshape(S, D), A_wqkv, A_wo, B_w1, B_b1.reshape(1, F), B_w2, B_b2.reshape(1, D), c, w_mod)
    return out.reshape(B, S, D)
```

```python
import jax
import jax.numpy as jnp
import jax.experimental.pallas as pl
import jax.experimental.pallas.tpu as pltpu

BF16 = jnp.bfloat16
F32 = jnp.float32
LOG2E = 1.4426950408889634

N_HEADS = 32
X1 = 128
XC = 512
BQ = 1024
BK = 128
OSPLIT = 2
FLAGS = {}
RB = 64
FLAT = False
HPI = 2
SAFE_RANGE = 200.0
SAFE_VMAX = 32768.0


def _ln(x):
    mu = jnp.mean(x, axis=-1, keepdims=True)
    xc = x - mu
    var = jnp.mean(xc * xc, axis=-1, keepdims=True)
    return xc * jax.lax.rsqrt(var + 1e-5)


def _nt(a, b):
    return jax.lax.dot_general(a, b, (((1,), (1,)), ((), ())), preferred_element_type=F32)


def _kernel(x_hbm, wqkv_hbm, wo_hbm, w1_hbm, b1_hbm, w2_hbm, b2_hbm, c_hbm, wmod_hbm,
            out_hbm,
            x_s, wqkv_s, wo_s, w1_s, w2_s, wmod_s, mod_s, h_s, k_s, qT_s, vT_s, oT_s,
            kp0, kp1, s0_s, m_s, x1_s, h2_s, out_s, c_ref, b1_ref, b2_ref, sems, osems, *, S, D, F, force_slow=False, dbg_iters=None):
    nx = S // XC
    dh = D // N_HEADS
    hpg = 128 // dh

    cp_mod0 = pltpu.make_async_copy(wmod_hbm.at[:, pl.ds(0, 2 * D)], wmod_s.at[:, pl.ds(0, 2 * D)], sems.at[0])

    def cp_w(j, si):
        return pltpu.make_async_copy(wqkv_hbm.at[:, pl.ds(j * D, D)], wqkv_s.at[:, pl.ds(j * D, D)], sems.at[si])

    cp_wq, cp_wk, cp_wv = cp_w(0, 1), cp_w(1, 2), cp_w(2, 3)
    xb = [0, X1] + [i * XC for i in range(1, nx + 1)] if X1 < XC else [i * XC for i in range(nx + 1)]
    cp_x = [pltpu.make_async_copy(x_hbm.at[pl.ds(a, b - a)], x_s.at[pl.ds(a, b - a)], sems.at[12 + i])
            for i, (a, b) in enumerate(zip(xb[:-1], xb[1:]))]
    cp_mod1 = pltpu.make_async_copy(wmod_hbm.at[:, pl.ds(2 * D, 4 * D)], wmod_s.at[:, pl.ds(2 * D, 4 * D)],
                                    sems.at[4])
    cp_wo = pltpu.make_async_copy(wo_hbm, wo_s, sems.at[5])
    cp_w1 = pltpu.make_async_copy(w1_hbm, w1_s, sems.at[6])
    cp_w2 = pltpu.make_async_copy(w2_hbm, w2_s, sems.at[7])
    cp_c = pltpu.make_async_copy(c_hbm, c_ref, sems.at[8])
    cp_b1 = pltpu.make_async_copy(b1_hbm, b1_ref, sems.at[9])
    cp_b2 = pltpu.make_async_copy(b2_hbm, b2_ref, sems.at[10])
    cp_c.start()
    cp_x[0].start()
    cp_mod0.start()
    cp_wk.start()
    order = cp_x[1:-1] + [cp_wq, cp_x[-1], cp_wv, cp_mod1, cp_wo, cp_b1, cp_b2, cp_w1, cp_w2]
    for cp in order:
        cp.start()

    cp_c.wait()
    cf = c_ref[...].astype(F32)
    sc = cf * jax.nn.sigmoid(cf)
    sc8 = jnp.broadcast_to(sc, (8, D)).astype(BF16)
    hh2, dd2 = N_HEADS // 2, D // 2
    r_id = jax.lax.broadcasted_iota(jnp.int32, (hh2, dd2), 0)
    c_id = jax.lax.broadcasted_iota(jnp.int32, (hh2, dd2), 1)
    e_mat = jnp.where((c_id // dh) == r_id, 1.0, 0.0).astype(BF16)
    qscale = (dh ** -0.5) * LOG2E

    cp_x[0].wait()
    cp_mod0.wait()
    mod0 = jnp.dot(sc8, wmod_s[:, 0:2 * D], preferred_element_type=F32)[0:1]
    sa = mod0[:, 0:D]
    ca1 = 1.0 + mod0[:, D:2 * D]

    kn_max = jnp.zeros((N_HEADS, 128), F32)

    def ln1(i):
        for r0 in range(i * X1, (i + 1) * X1, RB):
            rr = pl.ds(r0, RB)
            h_s[rr, :] = (_ln(x_s[rr, :].astype(F32)) * ca1 + sa).astype(BF16)
        return h_s[pl.ds(i * X1, X1), :]

    def stats_k(k2, kn_max):
        kn2 = jnp.concatenate([_nt(e_mat, k2[:, 0:dd2]), _nt(e_mat, k2[:, dd2:D])], axis=0)
        for t in range(k2.shape[0] // 128):
            kn_max = jnp.maximum(kn_max, kn2[:, t * 128:(t + 1) * 128])
        return kn_max

    hb_next = ln1(0)
    k2_prev = None
    n1 = S // X1
    for i in range(n1):
        hb = hb_next
        if i == 0:
            cp_wk.wait()
        if (i + 1) * X1 in xb[1:-1]:
            cp_x[xb.index((i + 1) * X1)].wait()
        if i == n1 - 2:
            cp_wq.wait()
            wqT = wqkv_s[:, 0:D].T
        kf = jnp.dot(hb, wqkv_s[:, D:2 * D], preferred_element_type=F32)
        if i == 0:
            kbar = jnp.sum(kf.reshape(X1 // 8, 8, D).sum(axis=0), axis=0, keepdims=True) * (1.0 / X1)
        kf = kf - kbar
        k_s[pl.ds(i * X1, X1), :] = kf.astype(BF16)
        if i + 1 < n1:
            hb_next = ln1(i + 1)
        if k2_prev is not None:
            kn_max = stats_k(k2_prev, kn_max)
        k2_prev = (kf * kf).astype(BF16)

    cp_wv.wait()
    wvT = wqkv_s[:, 2 * D:3 * D].T
    qn2 = []
    for i in range(nx):
        rows = pl.ds(i * XC, XC)
        qf = _nt(wqT, h_s[rows, :]) * qscale
        qT_s[:, rows] = qf.astype(BF16)
        if i == 0:
            kn_max = stats_k(k2_prev, kn_max)
            kn = jnp.max(kn_max, axis=1, keepdims=True)
        if i == nx - 1:
            cp_mod1.wait()
            mod1 = jnp.dot(sc8, wmod_s[:, 2 * D:6 * D], preferred_element_type=F32)[0:1]
            mod_s[...] = jnp.broadcast_to(mod1, (8, 4 * D))
        q2 = (qf * qf).astype(BF16)
        qn2.append(jnp.concatenate([jnp.dot(e_mat, q2[0:dd2], preferred_element_type=F32),
                                    jnp.dot(e_mat, q2[dd2:D], preferred_element_type=F32)], axis=0))

    vmax = jnp.zeros((8, 128), F32)
    spread = jnp.zeros((N_HEADS, XC), F32)
    for i in range(nx):
        rows = pl.ds(i * XC, XC)
        vf = _nt(wvT, h_s[rows, :])
        vT_s[:, rows] = vf.astype(BF16)
        ub = jnp.sqrt(qn2[i] * kn) * 1.02 + 1e-3
        m_s[:, rows] = ub * (0.5 - 1.0 / 128.0)
        spread = jnp.maximum(spread, ub)
        va = jnp.abs(vf)
        for t in range(XC // 128):
            vmax = jnp.maximum(vmax, va[:, t * 128:(t + 1) * 128].reshape(D // 8, 8, 128).max(axis=0))

    spread = jnp.max(jnp.max(spread, axis=1, keepdims=True), axis=0, keepdims=True)
    vm = jnp.max(jnp.max(vmax, axis=1, keepdims=True), axis=0, keepdims=True)
    ok = jnp.logical_and(spread * (1.0 + 1.0 / 64.0) <= SAFE_RANGE, vm <= SAFE_VMAX)
    safe = jnp.where(ok, 1, 0)[0, 0] > (1 if force_slow else 0)

    def prep(buf, h):
        g0 = pl.multiple_of((h // hpg) * 128, 128)
        kk = pltpu.bitcast(k_s[:, pl.ds(g0, 128)], jnp.uint32)
        kk = pltpu.roll(kk, (128 - (h % hpg) * dh) % 128, 1)
        buf[...] = pltpu.bitcast(kk, BF16)

    @pl.when(safe)
    def _fast():
        nq = S // BQ
        nk = S // BK
        bufs = (kp0, kp1)

        def qk(h, buf, j, c):
            h0 = pl.multiple_of(h * dh, dh)
            return jnp.dot(buf[c * BK:(c + 1) * BK, 0:dh], qT_s[pl.ds(h0, dh), j * BQ:(j + 1) * BQ],
                           preferred_element_type=F32)

        prep(kp0, 0)
        if FLAT:
            s0_s[...] = qk(0, kp0, 0, 0)

        def body(it, carry):
            items = [(u, j, c) for u in range(HPI) for j in range(nq) for c in range(nk)]
            hs = [it * HPI + u for u in range(HPI)] + [jnp.minimum(it * HPI + HPI, N_HEADS - 1)]
            pend = s0_s[...] if FLAT else qk(hs[0], bufs[0], 0, 0)
            acc = None
            l = None
            for i, (u, j, c) in enumerate(items):
                h = hs[u]
                h0 = pl.multiple_of(h * dh, dh)
                cols = slice(j * BQ, (j + 1) * BQ)
                if j == 0 and c == 0:
                    prep(bufs[(u + 1) % 2], hs[u + 1])
                sT = pend
                if i + 1 < len(items):
                    un, jn, cn = items[i + 1]
                    pend = qk(hs[un], bufs[un % 2], jn, cn)
                elif FLAT:
                    s0_s[...] = qk(hs[HPI], bufs[HPI % 2], 0, 0)
                p = jnp.exp2(sT - m_s[pl.ds(h, 1), cols])
                ps = p.reshape(BK // 8, 8, BQ).sum(axis=0)
                pv = jnp.dot(vT_s[pl.ds(h0, dh), pl.ds(c * BK, BK)], p.astype(BF16), preferred_element_type=F32)
                l = ps if c == 0 else l + ps
                acc = pv if c == 0 else acc + pv
                if c == nk - 1:
                    lt = jnp.sum(l, axis=0, keepdims=True)
                    oT_s[pl.ds(h0, dh), cols] = (acc * (1.0 / lt)).astype(BF16)
            return carry

        jax.lax.fori_loop(0, N_HEADS // HPI if dbg_iters is None else dbg_iters, body, 0)

    @pl.when(jnp.logical_not(safe))
    def _slow():
        bq, bk = 512, 256

        def hq_body(it, carry):
            h = it // (S // bq)
            j = it % (S // bq)
            h0 = pl.multiple_of(h * dh, dh)
            q0 = pl.multiple_of(j * bq, bq)
            prep(kp0, h)

            def k_body(c, st):
                m, l, acc = st
                k0 = pl.multiple_of(c * bk, bk)
                sT = jnp.dot(kp0[pl.ds(k0, bk), 0:dh], qT_s[pl.ds(h0, dh), pl.ds(q0, bq)],
                             preferred_element_type=F32)
                m_new = jnp.maximum(m, jnp.max(sT, axis=0, keepdims=True))
                alpha = jnp.exp2(m - m_new)
                p = jnp.exp2(sT - m_new)
                l = l * alpha + jnp.sum(p, axis=0, keepdims=True)
                acc = acc * alpha + jnp.dot(vT_s[pl.ds(h0, dh), pl.ds(k0, bk)], p.astype(BF16),
                                            preferred_element_type=F32)
                return m_new, l, acc

            m0 = jnp.full((1, bq), -jnp.inf, F32)
            _, l, acc = jax.lax.fori_loop(0, S // bk, k_body,
                                          (m0, jnp.zeros((1, bq), F32), jnp.zeros((dh, bq), F32)))
            oT_s[pl.ds(h0, dh), pl.ds(q0, bq)] = (acc / l).astype(BF16)
            return carry

        jax.lax.fori_loop(0, N_HEADS * (S // bq), hq_body, 0)

    ga = mod_s[0:1, 0:D]
    sb = mod_s[0:1, D:2 * D]
    cb1 = 1.0 + mod_s[0:1, 2 * D:3 * D]
    gb = mod_s[0:1, 3 * D:4 * D]
    cp_b1.wait()
    cp_b2.wait()
    cp_wo.wait()
    cp_w1.wait()
    cp_w2.wait()
    b1 = b1_ref[...].astype(F32).reshape(1, F)
    b2 = b2_ref[...].astype(F32).reshape(1, D)

    def proj(i):
        rows = pl.ds(i * XC, XC)
        a = jnp.dot(oT_s[:, rows].T, wo_s[...], preferred_element_type=F32)
        x1_s[i % 3] = x_s[rows, :].astype(F32) + ga * a

    def norm(i):
        for r0 in range(0, XC, RB):
            rr = pl.ds(r0, RB)
            h2_s[i % 2, rr, :] = (_ln(x1_s[i % 3, rr, :]) * cb1 + sb).astype(BF16)

    ocp = []
    proj(0)
    if nx > 1:
        proj(1)
    norm(0)
    for i in range(nx):
        rows = pl.ds(i * XC, XC)
        u = jnp.maximum(jnp.dot(h2_s[i % 2], w1_s[...], preferred_element_type=F32) + b1, 0.0)
        u = (u * u).astype(BF16)
        if i + 1 < nx:
            norm(i + 1)
        if i + 2 < nx:
            proj(i + 2)
        npc = OSPLIT if i == nx - 1 else 1
        pr = XC // npc
        for t in range(npc):
            prow = pl.ds(i * XC + t * pr, pr)
            y = jnp.dot(u[t * pr:(t + 1) * pr], w2_s[...], preferred_element_type=F32) + b2
            out_s[prow, :] = (x1_s[i % 3, t * pr:(t + 1) * pr, :] + gb * y).astype(BF16)
            cp = pltpu.make_async_copy(out_s.at[prow], out_hbm.at[prow], osems.at[i + t])
            cp.start()
            ocp.append(cp)
    for cp in ocp:
        cp.wait()


def _build(S, D, F, force_slow=False, dbg_iters=None):
    import functools
    nx = S // XC
    any_spec = pl.BlockSpec(memory_space=pl.ANY)
    return pl.pallas_call(
        functools.partial(_kernel, S=S, D=D, F=F, force_slow=force_slow, dbg_iters=dbg_iters),
        out_shape=jax.ShapeDtypeStruct((S, D), BF16),
        in_specs=[any_spec] * 9,
        out_specs=any_spec,
        scratch_shapes=[
            pltpu.VMEM((S, D), BF16),
            pltpu.VMEM((D, 3 * D), BF16),
            pltpu.VMEM((D, D), BF16),
            pltpu.VMEM((D, F), BF16),
            pltpu.VMEM((F, D), BF16),
            pltpu.VMEM((D, 6 * D), BF16),
            pltpu.VMEM((8, 4 * D), F32),
            pltpu.VMEM((S, D), BF16),
            pltpu.VMEM((S, D), BF16),
            pltpu.VMEM((D, S), BF16),
            pltpu.VMEM((D, S), BF16),
            pltpu.VMEM((D, S), BF16),
            pltpu.VMEM((S, 128), BF16),
            pltpu.VMEM((S, 128), BF16),
            pltpu.VMEM((BK, BQ), F32),
            pltpu.VMEM((N_HEADS, S), F32),
            pltpu.VMEM((3, XC, D), F32),
            pltpu.VMEM((2, XC, D), BF16),
            pltpu.VMEM((S, D), BF16),
            pltpu.VMEM((1, D), BF16),
            pltpu.VMEM((F,), BF16),
            pltpu.VMEM((D,), BF16),
            pltpu.SemaphoreType.DMA((13 + nx,)),
            pltpu.SemaphoreType.DMA((nx + OSPLIT - 1,)),
        ],
        compiler_params=pltpu.CompilerParams(vmem_limit_bytes=100 * 2 ** 20, **({"flags": FLAGS} if FLAGS else {})),
        name="adaln_block",
    )


@jax.jit
def pallas_adaLN_cond__mha_block__dense_activation_squared_relu__prompt_kernel(
    A_x: jax.Array,
    A_wqkv: jax.Array,
    A_wo: jax.Array,
    B_x: jax.Array,
    B_w1: jax.Array,
    B_b1: jax.Array,
    B_w2: jax.Array,
    B_b2: jax.Array,
    c: jax.Array,
    w_mod: jax.Array,
):
    del B_x
    B, S, D = A_x.shape
    F = B_w1.shape[1]
    out = _build(S, D, F)(
        A_x.reshape(S, D), A_wqkv, A_wo, B_w1, B_b1, B_w2, B_b2, c, w_mod)
    return out.reshape(B, S, D)
```

```python
import functools

import jax
import jax.numpy as jnp
import jax.experimental.pallas as pl
import jax.experimental.pallas.tpu as pltpu


BF16 = jnp.bfloat16
F32 = jnp.float32
LOG2E = 1.4426950408889634

N_HEADS = 32
X1 = 128
XC = 512
BQ = 512
BK = 128
OSPLIT = 2
RB = 64
PIPE = 3
HPI = 4
SAFE_RANGE = 200.0
SAFE_VMAX = 32768.0


def _ln(x):
    mu = jnp.mean(x, axis=-1, keepdims=True)
    xc = x - mu
    var = jnp.mean(xc * xc, axis=-1, keepdims=True)
    return xc * jax.lax.rsqrt(var + 1e-5)


def _nt(a, b):
    return jax.lax.dot_general(a, b, (((1,), (1,)), ((), ())), preferred_element_type=F32)


def _kernel(x_hbm, wqkv_hbm, wo_hbm, w1_hbm, b1_hbm, w2_hbm, b2_hbm, c_hbm, wmod_hbm,
            out_hbm,
            x_s, wqkv_s, wo_s, w1_s, w2_s, wmod_s, mod_s, h_s, k_s, qT_s, vT_s, oT_s,
            kp0, kp1, m_s, x1_s, h2_s, out_s, c_ref, b1_ref, b2_ref, sems, osems, *, S, D, F):
    nx = S // XC
    dh = D // N_HEADS
    hpg = 128 // dh

    cp_mod0 = pltpu.make_async_copy(wmod_hbm.at[:, pl.ds(0, 2 * D)], wmod_s.at[:, pl.ds(0, 2 * D)], sems.at[0])

    def cp_w(j, si):
        return pltpu.make_async_copy(wqkv_hbm.at[:, pl.ds(j * D, D)], wqkv_s.at[:, pl.ds(j * D, D)], sems.at[si])

    cp_wq, cp_wk, cp_wv = cp_w(0, 1), cp_w(1, 2), cp_w(2, 3)
    xb = [0, X1] + [i * XC for i in range(1, nx + 1)] if X1 < XC else [i * XC for i in range(nx + 1)]
    cp_x = [pltpu.make_async_copy(x_hbm.at[pl.ds(a, b - a)], x_s.at[pl.ds(a, b - a)], sems.at[12 + i])
            for i, (a, b) in enumerate(zip(xb[:-1], xb[1:]))]
    cp_mod1 = pltpu.make_async_copy(wmod_hbm.at[:, pl.ds(2 * D, 4 * D)], wmod_s.at[:, pl.ds(2 * D, 4 * D)],
                                    sems.at[4])
    cp_wo = pltpu.make_async_copy(wo_hbm, wo_s, sems.at[5])
    cp_w1 = pltpu.make_async_copy(w1_hbm, w1_s, sems.at[6])
    cp_w2 = pltpu.make_async_copy(w2_hbm, w2_s, sems.at[7])
    cp_c = pltpu.make_async_copy(c_hbm, c_ref, sems.at[8])
    cp_b1 = pltpu.make_async_copy(b1_hbm, b1_ref, sems.at[9])
    cp_b2 = pltpu.make_async_copy(b2_hbm, b2_ref, sems.at[10])
    cp_c.start()
    cp_x[0].start()
    cp_mod0.start()
    cp_wk.start()
    order = cp_x[1:-1] + [cp_wq, cp_x[-1], cp_wv, cp_mod1, cp_wo, cp_b1, cp_b2, cp_w1, cp_w2]
    for cp in order:
        cp.start()

    cp_c.wait()
    cf = c_ref[...].astype(F32)
    sc = cf * jax.nn.sigmoid(cf)
    sc8 = jnp.broadcast_to(sc, (8, D)).astype(BF16)
    hh2, dd2 = N_HEADS // 2, D // 2
    r_id = jax.lax.broadcasted_iota(jnp.int32, (hh2, dd2), 0)
    c_id = jax.lax.broadcasted_iota(jnp.int32, (hh2, dd2), 1)
    e_mat = jnp.where((c_id // dh) == r_id, 1.0, 0.0).astype(BF16)
    qscale = (dh ** -0.5) * LOG2E

    cp_x[0].wait()
    cp_mod0.wait()
    mod0 = jnp.dot(sc8, wmod_s[:, 0:2 * D], preferred_element_type=F32)[0:1]
    sa = mod0[:, 0:D]
    ca1 = 1.0 + mod0[:, D:2 * D]

    kn_max = jnp.zeros((N_HEADS, 128), F32)

    def ln1(i):
        for r0 in range(i * X1, (i + 1) * X1, RB):
            rr = pl.ds(r0, RB)
            h_s[rr, :] = (_ln(x_s[rr, :].astype(F32)) * ca1 + sa).astype(BF16)
        return h_s[pl.ds(i * X1, X1), :]

    def stats_k(k2, kn_max):
        kn2 = jnp.concatenate([_nt(e_mat, k2[:, 0:dd2]), _nt(e_mat, k2[:, dd2:D])], axis=0)
        for t in range(k2.shape[0] // 128):
            kn_max = jnp.maximum(kn_max, kn2[:, t * 128:(t + 1) * 128])
        return kn_max

    hb_next = ln1(0)
    k2_prev = None
    n1 = S // X1
    for i in range(n1):
        hb = hb_next
        if i == 0:
            cp_wk.wait()
        if (i + 1) * X1 in xb[1:-1]:
            cp_x[xb.index((i + 1) * X1)].wait()
        if i == n1 - 2:
            cp_wq.wait()
            wqT = wqkv_s[:, 0:D].T
        kf = jnp.dot(hb, wqkv_s[:, D:2 * D], preferred_element_type=F32)
        if i == 0:
            kbar = jnp.sum(kf.reshape(X1 // 8, 8, D).sum(axis=0), axis=0, keepdims=True) * (1.0 / X1)
        kf = kf - kbar
        k_s[pl.ds(i * X1, X1), :] = kf.astype(BF16)
        if i + 1 < n1:
            hb_next = ln1(i + 1)
        if k2_prev is not None:
            kn_max = stats_k(k2_prev, kn_max)
        k2_prev = (kf * kf).astype(BF16)

    cp_wv.wait()
    wvT = wqkv_s[:, 2 * D:3 * D].T
    qn2 = []
    for i in range(nx):
        rows = pl.ds(i * XC, XC)
        qf = _nt(wqT, h_s[rows, :]) * qscale
        qT_s[:, rows] = qf.astype(BF16)
        if i == 0:
            kn_max = stats_k(k2_prev, kn_max)
            kn = jnp.max(kn_max, axis=1, keepdims=True)
        q2 = (qf * qf).astype(BF16)
        qn2.append(jnp.concatenate([jnp.dot(e_mat, q2[0:dd2], preferred_element_type=F32),
                                    jnp.dot(e_mat, q2[dd2:D], preferred_element_type=F32)], axis=0))

    def prep(buf, h):
        g0 = pl.multiple_of((h // hpg) * 128, 128)
        kk = pltpu.bitcast(k_s[:, pl.ds(g0, 128)], jnp.uint32)
        kk = pltpu.roll(kk, (128 - (h % hpg) * dh) % 128, 1)
        buf[...] = pltpu.bitcast(kk, BF16)

    cp_mod1.wait()
    vmax = jnp.zeros((8, 128), F32)
    spread = jnp.zeros((N_HEADS, XC), F32)
    for i in range(nx):
        rows = pl.ds(i * XC, XC)
        vf = _nt(wvT, h_s[rows, :])
        vT_s[:, rows] = vf.astype(BF16)
        for b in range(i * 4 // nx, (i + 1) * 4 // nx):
            mod_s[:, b * D:(b + 1) * D] = jnp.dot(sc8, wmod_s[:, (2 + b) * D:(3 + b) * D], preferred_element_type=F32)
        if i == 0:
            kp0[...] = k_s[:, 0:128]
        ub = jnp.sqrt(qn2[i] * kn) * 1.02 + 1e-3
        m_s[:, rows] = ub * (0.5 - 1.0 / 128.0)
        spread = jnp.maximum(spread, ub)
        va = jnp.abs(vf)
        for t in range(XC // 128):
            vmax = jnp.maximum(vmax, va[:, t * 128:(t + 1) * 128].reshape(D // 8, 8, 128).max(axis=0))

    spread = jnp.max(jnp.max(spread, axis=1, keepdims=True), axis=0, keepdims=True)
    vm = jnp.max(jnp.max(vmax, axis=1, keepdims=True), axis=0, keepdims=True)
    ok = jnp.logical_and(spread * (1.0 + 1.0 / 64.0) <= SAFE_RANGE, vm <= SAFE_VMAX)
    safe = jnp.where(ok, 1, 0)[0, 0] > 0

    @pl.when(safe)
    def _fast():
        nq = S // BQ
        nk = S // BK
        bufs = (kp0, kp1)

        def qk(h, buf, j, c):
            h0 = pl.multiple_of(h * dh, dh)
            return jnp.dot(buf[c * BK:(c + 1) * BK, 0:dh], qT_s[pl.ds(h0, dh), j * BQ:(j + 1) * BQ],
                           preferred_element_type=F32)

        def body(it, carry):
            items = [(u, j, c) for u in range(HPI) for j in range(nq) for c in range(nk)]
            hs = [it * HPI + u for u in range(HPI)] + [jnp.minimum(it * HPI + HPI, N_HEADS - 1)]
            pend = [qk(hs[u], bufs[u % 2], j, c) for (u, j, c) in items[:PIPE]]
            acc = {}
            l = {}
            for i, (u, j, c) in enumerate(items):
                h = hs[u]
                h0 = pl.multiple_of(h * dh, dh)
                cols = slice(j * BQ, (j + 1) * BQ)
                if (j, c) == (0, 0):
                    prep(bufs[(u + 1) % 2], hs[u + 1])
                if i + PIPE < len(items):
                    un, jn, cn = items[i + PIPE]
                    pend.append(qk(hs[un], bufs[un % 2], jn, cn))
                sT = pend.pop(0)
                p = jnp.exp2(sT - m_s[pl.ds(h, 1), cols])
                ps = p.reshape(BK // 8, 8, BQ).sum(axis=0)
                pv = jnp.dot(vT_s[pl.ds(h0, dh), pl.ds(c * BK, BK)], p.astype(BF16), preferred_element_type=F32)
                l[j] = ps if c == 0 else l[j] + ps
                acc[j] = pv if c == 0 else acc[j] + pv
                if c == nk - 1:
                    lt = jnp.sum(l[j], axis=0, keepdims=True)
                    oT_s[pl.ds(h0, dh), cols] = (acc[j] * (1.0 / lt)).astype(BF16)
            return carry

        jax.lax.fori_loop(0, N_HEADS // HPI, body, 0)

    @pl.when(jnp.logical_not(safe))
    def _slow():
        bq, bk = 512, 256

        def hq_body(it, carry):
            h = it // (S // bq)
            j = it % (S // bq)
            h0 = pl.multiple_of(h * dh, dh)
            q0 = pl.multiple_of(j * bq, bq)
            prep(kp0, h)

            def k_body(c, st):
                m, l, acc = st
                k0 = pl.multiple_of(c * bk, bk)
                sT = jnp.dot(kp0[pl.ds(k0, bk), 0:dh], qT_s[pl.ds(h0, dh), pl.ds(q0, bq)],
                             preferred_element_type=F32)
                m_new = jnp.maximum(m, jnp.max(sT, axis=0, keepdims=True))
                alpha = jnp.exp2(m - m_new)
                p = jnp.exp2(sT - m_new)
                l = l * alpha + jnp.sum(p, axis=0, keepdims=True)
                acc = acc * alpha + jnp.dot(vT_s[pl.ds(h0, dh), pl.ds(k0, bk)], p.astype(BF16),
                                            preferred_element_type=F32)
                return m_new, l, acc

            m0 = jnp.full((1, bq), -jnp.inf, F32)
            _, l, acc = jax.lax.fori_loop(0, S // bk, k_body,
                                          (m0, jnp.zeros((1, bq), F32), jnp.zeros((dh, bq), F32)))
            oT_s[pl.ds(h0, dh), pl.ds(q0, bq)] = (acc / l).astype(BF16)
            return carry

        jax.lax.fori_loop(0, N_HEADS * (S // bq), hq_body, 0)

    ga = mod_s[0:1, 0:D]
    sb = mod_s[0:1, D:2 * D]
    cb1 = 1.0 + mod_s[0:1, 2 * D:3 * D]
    gb = mod_s[0:1, 3 * D:4 * D]
    cp_b1.wait()
    cp_b2.wait()
    cp_wo.wait()
    cp_w1.wait()
    cp_w2.wait()
    b1 = b1_ref[...].astype(F32).reshape(1, F)
    b2 = b2_ref[...].astype(F32).reshape(1, D)

    def proj(i):
        rows = pl.ds(i * XC, XC)
        a = jnp.dot(oT_s[:, rows].T, wo_s[...], preferred_element_type=F32)
        x1_s[i % 3] = x_s[rows, :].astype(F32) + ga * a

    def norm(i):
        for r0 in range(0, XC, RB):
            rr = pl.ds(r0, RB)
            h2_s[i % 2, rr, :] = (_ln(x1_s[i % 3, rr, :]) * cb1 + sb).astype(BF16)

    ocp = []
    proj(0)
    if nx > 1:
        proj(1)
    norm(0)
    for i in range(nx):
        rows = pl.ds(i * XC, XC)
        u = jnp.maximum(jnp.dot(h2_s[i % 2], w1_s[...], preferred_element_type=F32) + b1, 0.0)
        u = (u * u).astype(BF16)
        if i + 1 < nx:
            norm(i + 1)
        if i + 2 < nx:
            proj(i + 2)
        npc = OSPLIT if i == nx - 1 else 1
        pr = XC // npc
        for t in range(npc):
            prow = pl.ds(i * XC + t * pr, pr)
            y = jnp.dot(u[t * pr:(t + 1) * pr], w2_s[...], preferred_element_type=F32) + b2
            out_s[prow, :] = (x1_s[i % 3, t * pr:(t + 1) * pr, :] + gb * y).astype(BF16)
            cp = pltpu.make_async_copy(out_s.at[prow], out_hbm.at[prow], osems.at[i + t])
            cp.start()
            ocp.append(cp)
    for cp in ocp:
        cp.wait()


def _build(S, D, F):
    nx = S // XC
    any_spec = pl.BlockSpec(memory_space=pl.ANY)
    return pl.pallas_call(
        functools.partial(_kernel, S=S, D=D, F=F),
        out_shape=jax.ShapeDtypeStruct((S, D), BF16),
        in_specs=[any_spec] * 9,
        out_specs=any_spec,
        scratch_shapes=[
            pltpu.VMEM((S, D), BF16),
            pltpu.VMEM((D, 3 * D), BF16),
            pltpu.VMEM((D, D), BF16),
            pltpu.VMEM((D, F), BF16),
            pltpu.VMEM((F, D), BF16),
            pltpu.VMEM((D, 6 * D), BF16),
            pltpu.VMEM((8, 4 * D), F32),
            pltpu.VMEM((S, D), BF16),
            pltpu.VMEM((S, D), BF16),
            pltpu.VMEM((D, S), BF16),
            pltpu.VMEM((D, S), BF16),
            pltpu.VMEM((D, S), BF16),
            pltpu.VMEM((S, 128), BF16),
            pltpu.VMEM((S, 128), BF16),
            pltpu.VMEM((N_HEADS, S), F32),
            pltpu.VMEM((3, XC, D), F32),
            pltpu.VMEM((2, XC, D), BF16),
            pltpu.VMEM((S, D), BF16),
            pltpu.VMEM((1, D), BF16),
            pltpu.VMEM((F,), BF16),
            pltpu.VMEM((D,), BF16),
            pltpu.SemaphoreType.DMA((13 + nx,)),
            pltpu.SemaphoreType.DMA((nx + OSPLIT - 1,)),
        ],
        compiler_params=pltpu.CompilerParams(vmem_limit_bytes=100 * 2 ** 20),
        name="adaln_block",
    )


@jax.jit
def pallas_adaLN_cond__mha_block__dense_activation_squared_relu__prompt_kernel(
    A_x: jax.Array,
    A_wqkv: jax.Array,
    A_wo: jax.Array,
    B_x: jax.Array,
    B_w1: jax.Array,
    B_b1: jax.Array,
    B_w2: jax.Array,
    B_b2: jax.Array,
    c: jax.Array,
    w_mod: jax.Array,
):
    del B_x
    B, S, D = A_x.shape
    F = B_w1.shape[1]
    out = _build(S, D, F)(
        A_x.reshape(S, D), A_wqkv, A_wo, B_w1, B_b1, B_w2, B_b2, c, w_mod)
    return out.reshape(B, S, D)
```

```python
import functools

import jax
import jax.numpy as jnp
import jax.experimental.pallas as pl
import jax.experimental.pallas.tpu as pltpu


BF16 = jnp.bfloat16
F32 = jnp.float32
LOG2E = 1.4426950408889634

N_HEADS = 32
X1 = 128
X0 = 256
XC = 512
BQ = 512
BK = 128
OSPLIT = 2
RB = 64
PIPE = 3
HPI = 4
SAFE_RANGE = 200.0
SAFE_VMAX = 32768.0


def _ln(x):
    mu = jnp.mean(x, axis=-1, keepdims=True)
    xc = x - mu
    var = jnp.mean(xc * xc, axis=-1, keepdims=True)
    return xc * jax.lax.rsqrt(var + 1e-5)


def _nt(a, b):
    return jax.lax.dot_general(a, b, (((1,), (1,)), ((), ())), preferred_element_type=F32)


def _kernel(x_hbm, wqkv_hbm, wo_hbm, w1_hbm, b1_hbm, w2_hbm, b2_hbm, c_hbm, wmod_hbm,
            out_hbm,
            x_s, wqkv_s, wo_s, w1_s, w2_s, wmod_s, mod_s, h_s, k_s, qT_s, vT_s, oT_s,
            kp0, kp1, m_s, x1_s, h2_s, out_s, c_ref, b1_ref, b2_ref, sems, osems, *, S, D, F):
    nx = S // XC
    dh = D // N_HEADS
    hpg = 128 // dh

    cp_mod0 = pltpu.make_async_copy(wmod_hbm.at[:, pl.ds(0, 2 * D)], wmod_s.at[:, pl.ds(0, 2 * D)], sems.at[0])

    def cp_w(j, si):
        return pltpu.make_async_copy(wqkv_hbm.at[:, pl.ds(j * D, D)], wqkv_s.at[:, pl.ds(j * D, D)], sems.at[si])

    cp_wq, cp_wk, cp_wv = cp_w(0, 1), cp_w(1, 2), cp_w(2, 3)
    xb = [0, X0] + [i * XC for i in range(1, nx + 1)] if X0 < XC else [i * XC for i in range(nx + 1)]
    cp_x = [pltpu.make_async_copy(x_hbm.at[pl.ds(a, b - a)], x_s.at[pl.ds(a, b - a)], sems.at[12 + i])
            for i, (a, b) in enumerate(zip(xb[:-1], xb[1:]))]
    cp_mod1 = pltpu.make_async_copy(wmod_hbm.at[:, pl.ds(2 * D, 4 * D)], wmod_s.at[:, pl.ds(2 * D, 4 * D)],
                                    sems.at[4])
    cp_wo = pltpu.make_async_copy(wo_hbm, wo_s, sems.at[5])
    cp_w1 = pltpu.make_async_copy(w1_hbm, w1_s, sems.at[6])
    cp_w2 = pltpu.make_async_copy(w2_hbm, w2_s, sems.at[7])
    cp_c = pltpu.make_async_copy(c_hbm, c_ref, sems.at[8])
    cp_b1 = pltpu.make_async_copy(b1_hbm, b1_ref, sems.at[9])
    cp_b2 = pltpu.make_async_copy(b2_hbm, b2_ref, sems.at[10])
    cp_c.start()
    cp_x[0].start()
    cp_mod0.start()
    cp_wk.start()
    order = cp_x[1:] + [cp_wq, cp_wv, cp_mod1, cp_wo, cp_b1, cp_b2, cp_w1, cp_w2]
    for cp in order:
        cp.start()

    cp_c.wait()
    cf = c_ref[...].astype(F32)
    sc = cf * jax.nn.sigmoid(cf)
    sc8 = jnp.broadcast_to(sc, (8, D)).astype(BF16)
    hh2, dd2 = N_HEADS // 2, D // 2
    r_id = jax.lax.broadcasted_iota(jnp.int32, (hh2, dd2), 0)
    c_id = jax.lax.broadcasted_iota(jnp.int32, (hh2, dd2), 1)
    e_mat = jnp.where((c_id // dh) == r_id, 1.0, 0.0).astype(BF16)
    qscale = (dh ** -0.5) * LOG2E

    cp_x[0].wait()
    cp_mod0.wait()
    mod0 = jnp.dot(sc8, wmod_s[:, 0:2 * D], preferred_element_type=F32)[0:1]
    sa = mod0[:, 0:D]
    ca1 = 1.0 + mod0[:, D:2 * D]

    kn_max = jnp.zeros((N_HEADS, 128), F32)

    def ln1(i):
        for r0 in range(i * X1, (i + 1) * X1, RB):
            rr = pl.ds(r0, RB)
            h_s[rr, :] = (_ln(x_s[rr, :].astype(F32)) * ca1 + sa).astype(BF16)
        return h_s[pl.ds(i * X1, X1), :]

    def stats_k(k2, kn_max):
        kn2 = jnp.concatenate([_nt(e_mat, k2[:, 0:dd2]), _nt(e_mat, k2[:, dd2:D])], axis=0)
        for t in range(k2.shape[0] // 128):
            kn_max = jnp.maximum(kn_max, kn2[:, t * 128:(t + 1) * 128])
        return kn_max

    hb_next = ln1(0)
    k2_prev = None
    n1 = S // X1
    for i in range(n1):
        hb = hb_next
        if i == 0:
            cp_wk.wait()
        if (i + 1) * X1 in xb[1:-1]:
            cp_x[xb.index((i + 1) * X1)].wait()
        if (i + 1) * X1 == xb[-2]:
            cp_wq.wait()
            cp_wv.wait()
            wqT = wqkv_s[:, 0:D].T
            wvT = wqkv_s[:, 2 * D:3 * D].T
        kf = jnp.dot(hb, wqkv_s[:, D:2 * D], preferred_element_type=F32)
        if i == 0:
            kbar = jnp.sum(kf.reshape(X1 // 8, 8, D).sum(axis=0), axis=0, keepdims=True) * (1.0 / X1)
        kf = kf - kbar
        k_s[pl.ds(i * X1, X1), :] = kf.astype(BF16)
        if i + 1 < n1:
            hb_next = ln1(i + 1)
        if k2_prev is not None:
            kn_max = stats_k(k2_prev, kn_max)
        k2_prev = (kf * kf).astype(BF16)

    qn2 = []
    for i in range(nx):
        rows = pl.ds(i * XC, XC)
        qf = _nt(wqT, h_s[rows, :]) * qscale
        qT_s[:, rows] = qf.astype(BF16)
        if i == 0:
            kn_max = stats_k(k2_prev, kn_max)
            kn = jnp.max(kn_max, axis=1, keepdims=True)
        q2 = (qf * qf).astype(BF16)
        qn2.append(jnp.concatenate([jnp.dot(e_mat, q2[0:dd2], preferred_element_type=F32),
                                    jnp.dot(e_mat, q2[dd2:D], preferred_element_type=F32)], axis=0))

    def prep(buf, h):
        g0 = pl.multiple_of((h // hpg) * 128, 128)
        kk = pltpu.bitcast(k_s[:, pl.ds(g0, 128)], jnp.uint32)
        kk = pltpu.roll(kk, (128 - (h % hpg) * dh) % 128, 1)
        buf[...] = pltpu.bitcast(kk, BF16)

    cp_mod1.wait()
    vmax = jnp.zeros((8, 128), F32)
    bad = jnp.zeros((N_HEADS, XC), F32)
    for i in range(nx):
        rows = pl.ds(i * XC, XC)
        vf = _nt(wvT, h_s[rows, :])
        vT_s[:, rows] = vf.astype(BF16)
        for b in range(i * 4 // nx, (i + 1) * 4 // nx):
            mod_s[:, b * D:(b + 1) * D] = jnp.dot(sc8, wmod_s[:, (2 + b) * D:(3 + b) * D], preferred_element_type=F32)
        if i == 0:
            kp0[...] = k_s[:, 0:128]
        ub = jnp.sqrt(qn2[i] * kn) * 1.02 + 1e-3
        m_s[:, rows] = ub * (0.5 - 1.0 / 128.0)
        bad = jnp.maximum(bad, jnp.where(ub * (1.0 + 1.0 / 64.0) <= SAFE_RANGE, 0.0, 1.0))
        va = jnp.abs(vf)
        for t in range(XC // 128):
            vmax = jnp.maximum(vmax, va[:, t * 128:(t + 1) * 128].reshape(D // 8, 8, 128).max(axis=0))

    bad = jnp.max(jnp.max(bad, axis=1, keepdims=True), axis=0, keepdims=True)
    vm = jnp.max(jnp.max(vmax, axis=1, keepdims=True), axis=0, keepdims=True)
    ok = jnp.logical_and(bad <= 0.0, vm <= SAFE_VMAX)
    safe = jnp.where(ok, 1, 0)[0, 0] > 0

    @pl.when(safe)
    def _fast():
        nq = S // BQ
        nk = S // BK
        bufs = (kp0, kp1)

        def qk(h, buf, j, c):
            h0 = pl.multiple_of(h * dh, dh)
            return jnp.dot(buf[c * BK:(c + 1) * BK, 0:dh], qT_s[pl.ds(h0, dh), j * BQ:(j + 1) * BQ],
                           preferred_element_type=F32)

        def body(it, carry):
            items = [(u, j, c) for u in range(HPI) for j in range(nq) for c in range(nk)]
            hs = [it * HPI + u for u in range(HPI)] + [jnp.minimum(it * HPI + HPI, N_HEADS - 1)]
            pend = [qk(hs[u], bufs[u % 2], j, c) for (u, j, c) in items[:PIPE]]
            acc = {}
            l = {}
            for i, (u, j, c) in enumerate(items):
                h = hs[u]
                h0 = pl.multiple_of(h * dh, dh)
                cols = slice(j * BQ, (j + 1) * BQ)
                if (j, c) == (0, 0):
                    prep(bufs[(u + 1) % 2], hs[u + 1])
                if i + PIPE < len(items):
                    un, jn, cn = items[i + PIPE]
                    pend.append(qk(hs[un], bufs[un % 2], jn, cn))
                sT = pend.pop(0)
                p = jnp.exp2(sT - m_s[pl.ds(h, 1), cols])
                ps = p.reshape(BK // 8, 8, BQ).sum(axis=0)
                pv = jnp.dot(vT_s[pl.ds(h0, dh), pl.ds(c * BK, BK)], p.astype(BF16), preferred_element_type=F32)
                l[j] = ps if c == 0 else l[j] + ps
                acc[j] = pv if c == 0 else acc[j] + pv
                if c == nk - 1:
                    lt = jnp.sum(l[j], axis=0, keepdims=True)
                    oT_s[pl.ds(h0, dh), cols] = (acc[j] * (1.0 / lt)).astype(BF16)
            return carry

        jax.lax.fori_loop(0, N_HEADS // HPI, body, 0)

    @pl.when(jnp.logical_not(safe))
    def _slow():
        bq, bk = 512, 256

        def hq_body(it, carry):
            h = it // (S // bq)
            j = it % (S // bq)
            h0 = pl.multiple_of(h * dh, dh)
            q0 = pl.multiple_of(j * bq, bq)
            prep(kp0, h)

            def k_body(c, st):
                m, l, acc = st
                k0 = pl.multiple_of(c * bk, bk)
                sT = jnp.dot(kp0[pl.ds(k0, bk), 0:dh], qT_s[pl.ds(h0, dh), pl.ds(q0, bq)],
                             preferred_element_type=F32)
                m_new = jnp.maximum(m, jnp.max(sT, axis=0, keepdims=True))
                alpha = jnp.exp2(m - m_new)
                p = jnp.exp2(sT - m_new)
                l = l * alpha + jnp.sum(p, axis=0, keepdims=True)
                acc = acc * alpha + jnp.dot(vT_s[pl.ds(h0, dh), pl.ds(k0, bk)], p.astype(BF16),
                                            preferred_element_type=F32)
                return m_new, l, acc

            m0 = jnp.full((1, bq), -jnp.inf, F32)
            _, l, acc = jax.lax.fori_loop(0, S // bk, k_body,
                                          (m0, jnp.zeros((1, bq), F32), jnp.zeros((dh, bq), F32)))
            oT_s[pl.ds(h0, dh), pl.ds(q0, bq)] = (acc / l).astype(BF16)
            return carry

        jax.lax.fori_loop(0, N_HEADS * (S // bq), hq_body, 0)

    ga = mod_s[0:1, 0:D]
    sb = mod_s[0:1, D:2 * D]
    cb1 = 1.0 + mod_s[0:1, 2 * D:3 * D]
    gb = mod_s[0:1, 3 * D:4 * D]
    cp_b1.wait()
    cp_b2.wait()
    cp_wo.wait()
    cp_w1.wait()
    cp_w2.wait()
    b1 = b1_ref[...].astype(F32).reshape(1, F)
    b2 = b2_ref[...].astype(F32).reshape(1, D)

    def proj(i):
        rows = pl.ds(i * XC, XC)
        a = jnp.dot(oT_s[:, rows].T, wo_s[...], preferred_element_type=F32)
        x1_s[i % 3] = x_s[rows, :].astype(F32) + ga * a

    def norm(i):
        for r0 in range(0, XC, RB):
            rr = pl.ds(r0, RB)
            h2_s[i % 2, rr, :] = (_ln(x1_s[i % 3, rr, :]) * cb1 + sb).astype(BF16)

    ocp = []
    proj(0)
    if nx > 1:
        proj(1)
    norm(0)
    for i in range(nx):
        rows = pl.ds(i * XC, XC)
        u = jnp.maximum(jnp.dot(h2_s[i % 2], w1_s[...], preferred_element_type=F32) + b1, 0.0)
        u = (u * u).astype(BF16)
        if i + 1 < nx:
            norm(i + 1)
        if i + 2 < nx:
            proj(i + 2)
        npc = OSPLIT if i == nx - 1 else 1
        pr = XC // npc
        for t in range(npc):
            prow = pl.ds(i * XC + t * pr, pr)
            y = jnp.dot(u[t * pr:(t + 1) * pr], w2_s[...], preferred_element_type=F32) + b2
            out_s[prow, :] = (x1_s[i % 3, t * pr:(t + 1) * pr, :] + gb * y).astype(BF16)
            cp = pltpu.make_async_copy(out_s.at[prow], out_hbm.at[prow], osems.at[i + t])
            cp.start()
            ocp.append(cp)
    for cp in ocp:
        cp.wait()


def _build(S, D, F):
    nx = S // XC
    any_spec = pl.BlockSpec(memory_space=pl.ANY)
    return pl.pallas_call(
        functools.partial(_kernel, S=S, D=D, F=F),
        out_shape=jax.ShapeDtypeStruct((S, D), BF16),
        in_specs=[any_spec] * 9,
        out_specs=any_spec,
        scratch_shapes=[
            pltpu.VMEM((S, D), BF16),
            pltpu.VMEM((D, 3 * D), BF16),
            pltpu.VMEM((D, D), BF16),
            pltpu.VMEM((D, F), BF16),
            pltpu.VMEM((F, D), BF16),
            pltpu.VMEM((D, 6 * D), BF16),
            pltpu.VMEM((8, 4 * D), F32),
            pltpu.VMEM((S, D), BF16),
            pltpu.VMEM((S, D), BF16),
            pltpu.VMEM((D, S), BF16),
            pltpu.VMEM((D, S), BF16),
            pltpu.VMEM((D, S), BF16),
            pltpu.VMEM((S, 128), BF16),
            pltpu.VMEM((S, 128), BF16),
            pltpu.VMEM((N_HEADS, S), F32),
            pltpu.VMEM((3, XC, D), F32),
            pltpu.VMEM((2, XC, D), BF16),
            pltpu.VMEM((S, D), BF16),
            pltpu.VMEM((1, D), BF16),
            pltpu.VMEM((F,), BF16),
            pltpu.VMEM((D,), BF16),
            pltpu.SemaphoreType.DMA((13 + nx,)),
            pltpu.SemaphoreType.DMA((nx + OSPLIT - 1,)),
        ],
        compiler_params=pltpu.CompilerParams(vmem_limit_bytes=100 * 2 ** 20),
        name="adaln_block",
    )


@jax.jit
def pallas_adaLN_cond__mha_block__dense_activation_squared_relu__prompt_kernel(
    A_x: jax.Array,
    A_wqkv: jax.Array,
    A_wo: jax.Array,
    B_x: jax.Array,
    B_w1: jax.Array,
    B_b1: jax.Array,
    B_w2: jax.Array,
    B_b2: jax.Array,
    c: jax.Array,
    w_mod: jax.Array,
):
    del B_x
    B, S, D = A_x.shape
    F = B_w1.shape[1]
    out = _build(S, D, F)(
        A_x.reshape(S, D), A_wqkv, A_wo, B_w1, B_b1, B_w2, B_b2, c, w_mod)
    return out.reshape(B, S, D)
```
